```python
import os as _os
_os.environ.setdefault("JAX_PLATFORMS", "cpu")
import jax
import jax.numpy as jnp

def _softmax(x, axis=-1):
    return jax.nn.softmax(x, axis=axis)
def _gelu(x):
    return jax.nn.gelu(x, approximate=True)
def _silu(x):
    return jax.nn.silu(x)
def _sigmoid(x):
    return jax.nn.sigmoid(x)
def _layernorm(x, axis=-1, eps=1e-5):
    m = jnp.mean(x, axis=axis, keepdims=True)
    v = jnp.var(x, axis=axis, keepdims=True)
    return (x - m) / jnp.sqrt(v + eps)
def _scatter_add(tgt, idx, src, axis=0):
    return tgt.at[idx].add(src)
def _segment_sum(src, seg, n):
    return jax.ops.segment_sum(src, seg, n)
class _Rng:
    def __init__(self, key):
        self._k = key
    def _next(self):
        self._k, sub = jax.random.split(self._k)
        return sub
    def normal(self, shape):
        return jax.random.normal(self._next(), shape, dtype=jnp.bfloat16)
    def randint(self, lo, hi, shape):
        return jax.random.randint(self._next(), shape, lo, hi, dtype=jnp.int32)
    def uniform(self, shape, lo=0.0, hi=1.0):
        return jax.random.uniform(self._next(), shape, jnp.bfloat16, lo, hi)
    def permutation(self, n):
        return jax.random.permutation(self._next(), n)


kernel_name = 'interleave_layers__linear_kernel_hedgehog__sliding_block__prompt'

def setup_inputs():
    _rng = _Rng(jax.random.key(int.from_bytes(__import__("os").urandom(4), "little")))
    _w = (lambda a: (lambda t: t.astype(jnp.bfloat16) if jnp.issubdtype(t.dtype, jnp.floating) else t)(jnp.asarray(a)))
    def _A_setup():
        B, S, D, H = 1, 2048, 448, 16
        Dh = D // H
        return {
            "x": _w((lambda *s: _rng.normal(s) * 0.05)(B, S, D)),
            "wqkv": _w((lambda *s: _rng.normal(s) * 0.4)(D, 3 * D)),
            "w_phi": _w((lambda *s: _rng.normal(s) * 0.4)(H, Dh, Dh) * (Dh ** -0.5)),
            "wo": _w((lambda *s: _rng.normal(s) * 0.05)(D, D)),
        }
    _A_in = _A_setup()

    def _B_setup():
        B, S, D = 1, 2048, 448
        return {
            "x": _w((lambda *s: _rng.normal(s) * 0.05)(B, S, D)),
            "wqkv": _w((lambda *s: _rng.normal(s) * 0.1)(D, 3 * D)),
            "wo": _w((lambda *s: _rng.normal(s) * 0.1)(D, D)),
        }
    _B_in = _B_setup()

    return {
        "A_x": _A_in["x"],
        "A_wqkv": _A_in["wqkv"],
        "A_w_phi": _A_in["w_phi"],
        "A_wo": _A_in["wo"],
        "B_x": _B_in["x"],
        "B_wqkv": _B_in["wqkv"],
        "B_wo": _B_in["wo"],
    }

def reference(A_x, A_wqkv, A_w_phi, A_wo, B_x, B_wqkv, B_wo):
    def _A_ref(x, wqkv, w_phi, wo):
        B, S, D = x.shape
        H = 16; Dh = D // H
        qkv = (lambda x, *d: x.transpose(*d))((x @ wqkv).reshape(B, S, 3, H, Dh), 2, 0, 3, 1, 4)
        q, k, v = qkv[0], qkv[1], qkv[2]
        pq = jnp.einsum("bhsd,hdf->bhsf", q, w_phi)
        pk = jnp.einsum("bhsd,hdf->bhsf", k, w_phi)
        phi_q = jnp.concatenate([_softmax(pq, axis=-1), _softmax(-pq, axis=-1)], axis=-1)
        phi_k = jnp.concatenate([_softmax(pk, axis=-1), _softmax(-pk, axis=-1)], axis=-1)
        kv = jnp.einsum("bhsf,bhsd->bhfd", phi_k, v)
        z  = jnp.einsum("bhsf->bhf", phi_k)
        num = jnp.einsum("bhqf,bhfd->bhqd", phi_q, kv)
        den = jnp.einsum("bhqf,bhf->bhq", phi_q, z)[..., None] + 1e-6
        o = num / den
        return (lambda x, *d: x.transpose(*d))(o, 0, 2, 1, 3).reshape(B, S, D) @ wo

    def _B_ref(x, wqkv, wo):
        B, S, D = x.shape
        H = 16; Dh = D // H; W = 256
        qkv = (lambda x, *d: x.transpose(*d))((x @ wqkv).reshape(B, S, 3, H, Dh), 2, 0, 3, 1, 4)
        q, k, v = qkv[0], qkv[1], qkv[2]
        scores = jnp.einsum("bhqd,bhkd->bhqk", q, k) * (Dh ** -0.5)
        idx = jnp.arange(S)
        mask = (idx[:, None] - idx[None, :] >= 0) & (idx[:, None] - idx[None, :] < W)
        scores = jnp.where(mask[None, None], scores, -1e9)
        p = _softmax(scores, axis=-1)
        o = jnp.einsum("bhqk,bhkd->bhqd", p, v)
        return (lambda x, *d: x.transpose(*d))(o, 0, 2, 1, 3).reshape(B, S, D) @ wo

    x = A_x
    x = x + _A_ref(_layernorm(x, axis=-1), A_wqkv, A_w_phi, A_wo)
    x = x + _B_ref(_layernorm(x, axis=-1), B_wqkv, B_wo)
    x = x + _A_ref(_layernorm(x, axis=-1), A_wqkv, A_w_phi, A_wo)
    x = x + _B_ref(_layernorm(x, axis=-1), B_wqkv, B_wo)
    return x
```

```python
import math

import jax
import jax.numpy as jnp
from jax import lax
import jax.experimental.pallas as pl
import jax.experimental.pallas.tpu as pltpu

S, D, H, DH, WIN = 2048, 448, 16, 28, 256
DP = 512
T = 512
NC = S // T
LT = T // 128
PIECES = ((0, 8, 1, 2, 3, 4, 5, 6, 7),)
LAGS = (0, 0, 9, 23)
VSTEPS = (1, 3, 4, 5, 7, 8, 9, 11)
PHASE, HOLD = 1, 1
TIES, HEAVY, MEDIUM, LIGHT = (1, 4), (), (0, 4, 1, 5, 2), (3, 6, 2)
SWEEP_Q = ((0, 32), (32, 24))
FEATURES = "k0 k1 k2 k3 q0 s0 s1 q1 s2 s3"
LOG2E = math.log2(math.e)
NEG = -1e30
F32, BF16, I32 = jnp.float32, jnp.bfloat16, jnp.int32


def _iota(shape, dim):
    return lax.broadcasted_iota(I32, shape, dim)


def _dot(a, b):
    return jnp.dot(a, b, preferred_element_type=F32)


def _dot_nt(a, b):
    return lax.dot_general(a, b, (((1,), (1,)), ((), ())), preferred_element_type=F32)


def _tree(op, xs):
    xs = list(xs)
    while len(xs) > 1:
        xs = [op(xs[i], xs[i + 1]) if i + 1 < len(xs) else xs[i] for i in range(0, len(xs), 2)]
    return xs[0]


def _slabs(x):
    return [x[i:i + 8] for i in range(0, x.shape[0], 8)]


def _allreduce8(op, x, shifts=(4, 2, 1)):
    for s in shifts:
        x = op(x, pltpu.roll(x, s, 0))
    return x


def _pack(x):
    return pltpu.bitcast(x.astype(BF16), I32)


def _pack2(lo, hi):
    return pltpu.bitcast(pltpu.pack_elementwise([lo, hi], packed_dtype=BF16), I32)


def _zip(x):
    return jnp.concatenate([_pack2(x[i:i + 8], x[i + 8:i + 16]) for i in range(0, x.shape[0], 16)], axis=0)


def _unzip(words):
    lo, hi = pltpu.bitcast(words << 16, F32), pltpu.bitcast(words & -65536, F32)
    return jnp.concatenate([v[i:i + 8] for i in range(0, words.shape[0], 8) for v in (lo, hi)], axis=0)


def _mat(*words):
    return pltpu.bitcast(words[0] if len(words) == 1 else jnp.concatenate(words, axis=0), BF16)


def _recip(x):
    r = pl.reciprocal(x, approx=True)
    return r * (2.0 - x * r)


def _moments(x):
    xs = _slabs(x)
    mean = _tree(jnp.add, xs) * (1.0 / len(xs))
    return jnp.concatenate([mean, _tree(jnp.add, [(v - mean) * (v - mean) for v in xs])], axis=0)


def _hedgehog(p):
    ps = _slabs(p)
    mx = _allreduce8(jnp.maximum, _tree(jnp.maximum, ps), (4, 2))
    mn = _allreduce8(jnp.minimum, _tree(jnp.minimum, ps), (4, 2))
    es = [jnp.exp2(v - mx) for v in ps], [jnp.exp2(mn - v) for v in ps]
    sums = [_allreduce8(jnp.add, _tree(jnp.add, e), (4, 2)) for e in es]
    r = _recip(sums[0] * sums[1])
    return _pack2(*[jnp.concatenate([v * scale for v in e], axis=0) for e, scale in zip(es, (r * sums[1], r * sums[0]))])


def _attention_order(x):
    even = (_iota((8, x.shape[1]), 0) & 1) == 0
    out = []
    for r in range(0, x.shape[0], 2 * DH):
        s = _slabs(_mat(_zip(jnp.concatenate([x[r:r + 32], x[r + 24:r + 56]], axis=0))).astype(F32))
        out += s[:3] + [jnp.where(even, s[3], s[4])] + s[5:]
    return jnp.concatenate(out, axis=0)


def _transpose_block(src, j, row_order=None):
    w = min(128, src.shape[1] - 128 * j)
    blk = src[:, 128 * j:128 * j + w]
    if row_order:
        blk = _mat(_zip(row_order(blk.astype(F32))))
    blk = jnp.concatenate([blk, jnp.zeros((DP - D, w), BF16)], axis=0)
    if w < 128:
        blk = jnp.concatenate([blk, jnp.zeros((DP, 128 - w), BF16)], axis=1)
    words = pltpu.bitcast(blk.T, I32)[:w // 2]
    return _pack(_unzip(words)) if row_order else words


def _phi_blocks(phi_in, phi_a, phi_b):
    col = _iota((DH, 128), 1)
    sel = ((col % (2 * DH)) // 2 == _iota((DH, 128), 0)) & (col < 4 * DH)
    phi_a[...] = _dot(phi_in[...], jnp.where(sel, 1.0, 0.0).astype(BF16))
    for h in range(H):
        phi_b[h * DH:(h + 1) * DH, :] = phi_a[pl.ds(h, DH, stride=H), :]
    row, col = _iota((128, 128), 0), _iota((128, 128), 1)
    same_head = row // DH == (col // (2 * DH)) * 2 + col % 2
    out = []
    for b in range(4):
        m = jnp.concatenate([phi_b[112 * b:112 * (b + 1), :], jnp.zeros((16, 128), F32)], axis=0)
        out.append(jnp.where(same_head, m, 0.0).T[:112].astype(BF16))
    return out


def merge(a, b):
    keyed = [((i + 0.5) / len(a), i, x) for i, x in enumerate(a)] + [((i + 0.6) / len(b), i, x) for i, x in enumerate(b)]
    return [x for _, _, x in sorted(keyed, key=lambda k: k[:2])]


class _Buffer:
    def __init__(self, ref, rd):
        self.w, self.r, self.n = ref.at[0], ref.at[rd], ref.shape[2] - 8
        self.w[0, self.n:, :] = jnp.zeros((8, 128), I32)

    def load(self, start, size, lanes=slice(0, 512)):
        tiles = range(lanes.start // 128, lanes.stop // 128)
        return jnp.concatenate([self.r[j, start:start + size, :] for j in tiles], axis=1)

    def store(self, start, value, first_tile=0):
        for j in range(value.shape[1] // 128):
            self.w[first_tile + j, start:start + value.shape[0], :] = value[:, 128 * j:128 * (j + 1)]
        return self.r[0, self.n:, :]


def _kernel(x_hbm, wa_hbm, phi_hbm, woa_hbm, wb_hbm, wob_hbm, out_hbm,
            xin, wa_in, phi_in, woa_in, wb_in, wob_in, phi_a, phi_b, kv, kvb, ktail, qmask,
            in_sem, out_sem, weights, chunks, ws):
    def x_copy(c):
        return pltpu.make_async_copy(x_hbm.at[:, pl.ds(c * T, T)], xin.at[c], in_sem.at[c])

    def out_copy(c, b):
        rows = pl.ds(112 * b, 112)
        return pltpu.make_async_copy(xin.at[c, rows], out_hbm.at[rows, pl.ds(c * T, T)], out_sem.at[4 * c + b])

    columns = lambda a, b: (wa_hbm.at[:, pl.ds(a, b - a)], wa_in.at[:, pl.ds(a, b - a)])
    phi_copy, wv_copy, wk_copy, wq_copy, *w_copies = [
        pltpu.make_async_copy(s, d, in_sem.at[NC + i]) for i, (s, d) in enumerate((
            (phi_hbm, phi_in), columns(896, 3 * D), columns(384, 896), columns(0, 384),
            (woa_hbm, woa_in), (wb_hbm, wb_in), (wob_hbm, wob_in)))]
    for cp in (phi_copy, x_copy(0), wv_copy):
        cp.start()

    wr, rd = _iota((8, 128), 0)[0, 0], _iota((8, 128), 1)[0, 0]
    wa, woa, wb, wob, (pairs_a, pairs_b) = ([_Buffer(r, rd) for r in group] for group in weights)
    xs, xa, xb, phiq, oa, qt, ks, vt, ob, phik, va = ([_Buffer(r, rd) for r in group] for group in chunks)
    sub8 = _iota((8, T), 0)
    lane16 = _iota((16, 128), 1)
    tile = lambda j: slice(128 * j, 128 * (j + 1))
    zeros = lambda rows, lanes=128: jnp.zeros((rows, lanes), I32)
    background, companion = [], []

    def finish(buf):
        while any(dst is buf for dst, _ in background):
            for _ in background.pop(0)[1]:
                pass

    def tie():
        while background:
            for value in background[0][1]:
                return value if value.dtype == I32 else pltpu.bitcast(value, I32) & qmask[rd, 0, 3]
            background.pop(0)

    def proj(w, b, x, ties=TIES):
        finish(w)
        finish(x)
        out = []
        for j in range(LT):
            lhs = _slabs(w.load(56 * b, 56))
            for i in ties:
                z = tie()
                if z is not None:
                    lhs[i] = jnp.concatenate([lhs[i][:, :128] | z, lhs[i][:, 128:]], axis=1)
            out.append(_dot(_mat(*lhs), _mat(x.load(0, D // 2, tile(j)), zeros((DP - D) // 2))))
            if companion and j == LT - 1:
                run(companion.pop(0))
        return jnp.concatenate(out, axis=1)

    def proj_pair(w, b, x, ties, sweeps=((0, 56),)):
        finish(w)
        finish(x)
        top, bottom = [], []
        for j in range(LT // 2):
            parts = []
            for r0, rows in sweeps:
                m = {}
                for n in (0, 3, 4, 6, 1, 2, 5):
                    lhs = w.load(56 * (4 * b + n // 2) + r0, rows, slice(256 * (n % 2), 256 * (n % 2) + 256))
                    z = tie() if n in ties else None
                    if z is not None:
                        lhs = jnp.concatenate([jnp.concatenate([lhs[:8, :128] | z, lhs[:8, 128:]], axis=1), lhs[8:]], axis=0)
                    m[n] = _dot(_mat(lhs), _mat(x.load(128 * (n // 2), 128, tile(2 * j + n % 2))))
                parts.append((m[0] + m[3] - m[4] + m[6], m[4] + m[2], m[3] + m[1], m[0] - m[1] + m[2] + m[5]))
            c11, c12, c21, c22 = (jnp.concatenate(p, axis=0) for p in zip(*parts))
            top += [c11, c12]
            bottom += [c21, c22]
            if companion:
                run(companion.pop(0))
        return jnp.concatenate(top, axis=1), jnp.concatenate(bottom, axis=1)

    def store_x(c, b, x):
        return xs[c].store(128 * b, pltpu.bitcast(jnp.concatenate([x, _moments(x)], axis=0), I32))

    def normalize(c, dst):
        background.extend((dst[c], normalize_pair(c, j, dst)) for j in range(LT // 2))

    def normalize_pair(c, j, dst):
        for u in range(2):
            yield next(normalize_tile(c, 2 * j + u, dst))
        for r in range(0, 256, 32):
            stats = [_slabs(pltpu.bitcast(dst[c].load(dst[c].n - 16, 16, tile(2 * j + u)), F32)) for u in range(2)]

            def rows(r0, u):
                x = [xs[c].load(r + 16 * (r // 112), 8, tile(2 * j + u)) for r in range(r0, r0 + 32, 8)]
                return jnp.concatenate([(pltpu.bitcast(v, F32) - stats[u][0]) * stats[u][1] for v in x], axis=0)

            b11, b12 = rows(r, 0), rows(r, 1)
            if 256 + r < D:
                b21, b22 = rows(256 + r, 0), rows(256 + r, 1)
                ops = [b11 + b22, b11, b12 - b22, b21 - b11, b22, b11 + b12, b21 + b22]
            else:
                ops = [b11, b11, b12, -b11, jnp.zeros_like(b11), b11 + b12, jnp.zeros_like(b11)]
            for n, v in enumerate(ops):
                z = dst[c].store(128 * (n // 2) + r // 2, _zip(v), 2 * j + n % 2)
            yield z

    def normalize_tile(c, j, dst):
        m = [pltpu.bitcast(v, F32) for b in range(4) for v in _slabs(xs[c].load(128 * b + 112, 16, tile(j)))]
        mean = _allreduce8(jnp.add, _tree(jnp.add, m[0::2])) * (1.0 / 32)
        dev = _tree(jnp.add, m[1::2]) + 14.0 * _tree(jnp.add, [(v - mean) * (v - mean) for v in m[0::2]])
        r = lax.rsqrt(_allreduce8(jnp.add, dev) * (1.0 / D) + 1e-5)
        yield dst[c].store(dst[c].n - 16, pltpu.bitcast(jnp.concatenate([mean, r], axis=0), I32), j)
        for b in range(4):
            mean, r = _slabs(pltpu.bitcast(dst[c].load(dst[c].n - 16, 16, tile(j)), F32))
            x = _slabs(pltpu.bitcast(xs[c].load(128 * b, 112, tile(j)), F32))
            yield dst[c].store(56 * b, _zip(jnp.concatenate([(v - mean) * r for v in x], axis=0)), j)

    def residual(c, b, w, o):
        return pltpu.bitcast(xs[c].load(128 * b, 112), F32) + proj(w[0], b, o[c])

    def store_features(dst, b, p):
        return dst.store(112 * b, jnp.concatenate([_hedgehog(p[r:r + 56]) for r in range(0, p.shape[0], 56)], axis=0))

    def store_values(c, b, v):
        ones = jnp.ones((8, T), F32)
        va[4 * c + b].store(0, _zip(jnp.concatenate([v[:56], ones, v[56:], ones], axis=0)))

    def a_keys(c, b):
        k, v = proj_pair(pairs_a, b, xa[c], MEDIUM if c < NC - 1 else LIGHT)
        store_features(phik[4 * c + b], 0, k)
        store_values(c, b, v)

    def a_q(c, b):
        store_features(phiq[c], 2 * b, jnp.concatenate(proj_pair(pairs_a, 4 + b, xa[c], HEAVY, SWEEP_Q), axis=0))

    def a_kv(c, b):
        for g in (2 * b, 2 * b + 1):
            acc = _dot_nt(_mat(va[4 * c + b].load(32 * (g % 2), 32)), _mat(phik[4 * c + b].load(56 * (g % 2), 56), zeros(8, T)))
            if c > 0:
                acc += kv[rd, g]
            if c < NC - 1:
                kv[wr, g] = acc
            else:
                row, col = _iota((64, 128), 0), _iota((64, 128), 1)
                second = ((row >= DH) & (row < 2 * DH)) | (row >= 2 * DH + 4)
                kvb[wr, g] = _pack(jnp.where(second == ((col & 2) == 2), _unzip(_pack(acc)), 0.0))

    def a_features(c):
        tasks = [({"k": a_keys, "q": a_q, "s": a_kv}[name], c, int(b)) for name, b in FEATURES.split()]
        return [task for task in tasks if task != (a_q, NC - 1, 1)]

    def a_mix(c, b):
        o = []
        for g in (2 * b, 2 * b + 1):
            nd = _slabs(_dot(_mat(kvb[rd, g]), _mat(phiq[c].load(56 * g, 56), zeros(8, T))))
            r = _recip(nd[7] + 1e-6)
            rr = pltpu.roll(r, 4, 0)
            r0, r1 = jnp.where(sub8 < 4, r, rr), jnp.where(sub8 < 4, rr, r)
            o += [n * s for n, s in zip(nd, (r0, r0, r0, r, r1, r1, r1))]
        oa[c].store(56 * b, _zip(jnp.concatenate(o, axis=0)))

    def a_out(c, b):
        store_x(c, b, residual(c, b, woa, oa))
        if b == 3:
            normalize(c, xb)

    def b_qk(c, g):
        k, q = proj_pair(pairs_b, g, xb[c], (2,))
        q = q * (DH ** -0.5 * LOG2E)
        qt[c].store(56 * g, _pack2(q[:56], q[56:]))
        k = _pack2(k[:56], k[56:])
        odd, high = lane16 >= 2 * DH, (lane16 & 1) == 1
        kb = [ktail[rd, g, 16 * j:16 * j + 16] if c else zeros(16) for j in range(3)]
        x = [[jnp.where(odd, kb[j + 1 - b0], kb[j + b0]) for j in range(2)] for b0 in range(2)]
        for j in range(T // 32):
            if j % 4 == 0:
                kn = pltpu.bitcast(_mat(k[:, tile(j // 4)], zeros(8)).T, I32)
            kb.append(_pack(_unzip(kn[16 * (j % 4):16 * (j % 4) + 16])))
            if c < NC - 1 and j >= T // 32 - 3:
                ktail[wr, g, 16 * (j + 3 - T // 32):16 * (j + 4 - T // 32)] = kb[-1]
            for b0 in range(2):
                x[b0].append(jnp.where(odd, kb[j + 3 - b0], kb[j + 2 + b0]))
            y = [jnp.where(high, x[t & 1][j + 2 - (t & 2)], x[t & 1][j + (t & 2)]) for t in range(4)]
            ks[c].store(g * T // 2 + 16 * j, jnp.concatenate(y, axis=1))

    def b_v(c, g):
        v = _slabs(jnp.concatenate(proj_pair(pairs_b, 4 + g, xb[c], LIGHT), axis=0))
        rows = []
        for w in (v[:7], v[7:14], v[14:21], v[21:]):
            rows += w[0:3] + [jnp.where(sub8 < 4, w[3], 1.0), jnp.where(sub8 < 4, 1.0, w[3])] + w[4:7]
        vt[c].store(128 * g, _zip(jnp.concatenate(rows, axis=0)))

    def first_block(i):
        return max(0, 5 - 4 * i)

    def recent_mask():
        row, lane = _iota((32, 128), 0), _iota((32, 128), 1)
        return (row & 16) + 2 * (row & 7) + ((row >> 3) & 1) <= (lane & 31)

    def b_scores(c, g, j, out):
        i = c * LT + j
        for piece in PIECES:
            blocks = [n for n in piece if n >= first_block(i)]
            if blocks:
                pad, q = zeros(8), qt[c].load(56 * g, 56, tile(j))
            for t in range(4 if blocks else 0):
                k = [divmod(4 * i + n - 5, T // 32) for n in blocks]
                k = [ks[kc].load(g * T // 2 + 16 * kb, 16, tile(t)) for kc, kb in k]
                mask = [qmask[rd, t, r] for r in range(3)]
                d = _dot(_mat(*k), _mat(q & jnp.concatenate([mask[r] for r in (0, 0, 0, 1, 2, 2, 2)], axis=0), pad))
                out[t].update({n: d[32 * r:32 * r + 32] for r, n in enumerate(blocks)})
            for n in piece:
                yield

    def b_max(c, g, j, s, wr):
        i = c * LT + j
        m = [None] * 4
        for piece in PIECES:
            for n in piece:
                for t in range(4 if n >= max(1, first_block(i)) else 0):
                    v = s[t][n]
                    if n < 8 - 4 * i:
                        v = jnp.where(_iota((32, 128), 1) >= 32 * (8 - 4 * i - n), v, NEG)
                    if n == 8:
                        v = jnp.where(recent_mask(), v, s[t].get(0, NEG))
                    wr[t, 32 * n:32 * n + 32, :] = pltpu.bitcast(v, I32)
                    v = _tree(jnp.maximum, _slabs(v))
                    m[t] = v if m[t] is None else jnp.maximum(m[t], v)
                    if n == 7:
                        wr[t, 0:8, :] = pltpu.bitcast(_allreduce8(jnp.maximum, m[t]), I32)
                yield

    def b_exp(c, g, j, rd, out):
        n0 = first_block(c * LT + j)
        m = [jnp.concatenate([pltpu.bitcast(rd[t, 0:8, :], F32)] * 4, axis=0) for t in range(4)]
        for n in (8, 1, 2, 3, 4, 5, 6, 7):
            e = [jnp.exp2(pltpu.bitcast(rd[t, 32 * n:32 * n + 32, :], F32) - m[t]) for t in range(4 if n >= n0 else 0)]
            yield
            if n == 8 and n0 == 0:
                parts = {0: [jnp.where(recent_mask(), 0.0, v) for v in e], 8: [jnp.where(recent_mask(), v, 0.0) for v in e]}
            else:
                parts = {n: e}
            for b, vs in parts.items():
                out[b] = [_zip(v) for v in vs]
        yield

    def b_values(c, g, j, probs):
        i = c * LT + j
        n0 = first_block(i)
        zero = [jnp.zeros((16, 128), I32)] * 4
        odd, high = (lane16 & 32) != 0, (lane16 & 64) != 0
        p, u, ph, acc = zero, [zero, zero], [], [None] * 4
        for n in range(12):
            before, p = p, zero
            if n0 <= n < 9:
                p = probs[n]
            u.append([jnp.where(odd, before[t ^ 1], p[t]) for t in range(4)] if n0 <= n < 10 else zero)
            ph.append([jnp.where(high, u[-3][h ^ 2], u[-1][h]) for h in range(4)])
            vc, vj = divmod(i - 2 + n // 4, LT)
            if n % 4 == 3 and vc >= 0:
                for h in range(4):
                    d = _dot(_mat(vt[vc].load(16 * (4 * g + h), 16, tile(vj))), _mat(*[x[h] for x in ph[-4:]]))
                    acc[h] = d if acc[h] is None else acc[h] + d
            if n in VSTEPS:
                yield
        lo = (_iota((8, 128), 0) & 1) == 0
        o = []
        for a, b in (map(_slabs, acc[0:2]), map(_slabs, acc[2:4])):
            rr = _recip(jnp.where(lo, b[0], a[3]))
            r = pltpu.roll(rr, 1, 0)
            r0, r1 = jnp.where(lo, r, rr), jnp.where(lo, rr, r)
            o += [v * r0 for v in a[0:3]] + [jnp.where(lo, a[3], b[0]) * r] + [v * r1 for v in b[1:4]]
        ob[c].store(56 * g, _zip(jnp.concatenate(o, axis=0)), j)
        yield

    def b_out(c, b, final):
        x = residual(c, b, wob, ob)
        if final:
            xin[c, 112 * b:112 * (b + 1), :] = _mat(_zip(x))
            out_copy(c, b).start()
        else:
            store_x(c, b, x)
            if b == 3:
                normalize(c, xa)

    def run(tasks):
        for fn, *args in tasks:
            fn(*args)

    def section(tasks):
        pl.when(rd == 0)(lambda: run(tasks))

    def mix_and_attend(final):
        four = lambda fn, c, *args: [(fn, c, b, *args) for b in range(4)]
        b_inputs = lambda c: four(b_qk, c) + four(b_v, c)[:2]
        b_outputs = lambda c: four(b_out, c, final)
        run(four(a_mix, 0) + [(a_q, NC - 1, 1)] + merge(four(a_out, 0), four(a_mix, 1)) + four(a_out, 1))
        run(merge(b_inputs(0), four(a_mix, 2)))
        stages, fills = {}, []
        for c in range(NC):
            big = four(a_out, c + 2) if c + 2 < NC else b_outputs(c - 2)
            if c < NC - 1:
                inputs = b_inputs(c + 1)
                fill = big + inputs[:4] + merge(four(a_mix, c + 3) if c + 3 < NC else [], inputs[4:])
            else:
                fill = big + b_outputs(c - 1)[:HOLD]
            fills.append(fill)
            for n, unit in enumerate((c, g, j) for j in range(LT) for g in range(4)):
                s, p, w, r = [{} for _ in range(4)], {}, *[ws[(c * 4 * LT + n) % len(ws)].at[z] for z in (0, rd)]
                gens = (b_scores(*unit, s), b_max(*unit, s, w), b_exp(*unit, r, p), b_values(*unit, p))
                for order, (gen, lag) in enumerate(zip(gens, LAGS)):
                    for step in range(9):
                        stages.setdefault(36 * LT * c + 9 * n + lag + step, []).append((order, (next, gen)))
        rest = b_outputs(NC - 2)[HOLD:]
        steps = [[task for _, task in sorted(stages[step], key=lambda x: x[0])] for step in sorted(stages)]
        for fill in fills + [rest]:
            now, steps = steps[:36 * LT], steps[36 * LT:]
            slots = sum((task[0] is not a_mix) + (task[0] in (b_qk, b_v)) for task in fill)
            cuts = [max(0, len(now) * n // max(slots, 1) + PHASE) for n in range(slots)] + [len(now)]
            run(sum(now[:cuts[0]], []))
            companion.extend(sum(now[a:b], []) for a, b in zip(cuts, cuts[1:]))
            run(fill)
        run(b_outputs(NC - 1))
        if not final:
            for c in range(NC):
                (section if c < 2 else run)(a_features(c))

    def load_x(c):
        def pieces():
            for j in range(LT):
                for b in range(4):
                    x = _unzip(pltpu.bitcast(xin[c, 112 * b:112 * (b + 1), tile(j)], I32))
                    yield xs[c].store(128 * b, pltpu.bitcast(jnp.concatenate([x, _moments(x)], axis=0), I32), j)

        background.append((xs[c], pieces()))
        if c:
            normalize(c, xa)
        else:
            background.extend((xa[c], normalize_tile(c, j, xa)) for j in range(LT))

    def transpose(src, dst, row_order=None):
        def pieces():
            for j in range(pl.cdiv(src.shape[1], 128)):
                words = _transpose_block(src, j, row_order)
                for r in range(0, words.shape[0], 32):
                    part, row = divmod(64 * j + r, D // 2)
                    yield dst[part].store(row, words[r:r + 32])

        background.extend([(dst[0], pieces())] + [(buf, iter(())) for buf in dst[1:]])

    def pair_weights(w, dst, other):
        for b in range(6):
            for r in range(0, 56, 8):
                blocks = ((1, b), (other, b)) if b < 4 else ((2 - other, 2 * b - 8), (2 - other, 2 * b - 7))
                (a11, a12), (a21, a22) = (jnp.split(_unzip(w[p].load(56 * i + r, 8)), 2, axis=1) for p, i in blocks)
                for n, v in enumerate([a11 + a22, a21 + a22, a11, a22, a11 + a12, a21 - a11, a12 - a22]):
                    z = dst.store(56 * (4 * b + n // 2) + r, _zip(v), 2 * (n % 2))
                yield z

    qmask[wr, 0, 3] = zeros(8)
    for r in range(3):
        head = jnp.where(_iota((8, 128), 0) + 8 * (r + 2) >= DH, 1, 0) ^ (_iota((8, 128), 1) >> 5)
        for t in range(4):
            qmask[wr, t, r] = jnp.where(head == t, 65535, jnp.where(head == t ^ 2, -65536, 0))
    phi_copy.wait()
    phi = _phi_blocks(phi_in, phi_a, phi_b)
    x_copy(0).wait()
    wk_copy.start()
    x_copy(1).start()
    load_x(0)
    finish(xa[0])
    wv_copy.wait()
    wq_copy.start()
    wa[2].store(0, jnp.concatenate([_transpose_block(wa_in, j) for j in range(7, 11)], axis=0))
    wt = {}

    def fold(part, b):
        r0 = part * D // 2 + 56 * b
        for j in range(r0 // 64, (r0 + 55) // 64 + 1):
            if j not in wt:
                wt[j] = _transpose_block(wa_in, j)
        rows = [wt[r // 64][r % 64:r % 64 + 8] for r in range(r0, r0 + 56, 8)]
        wa[part].store(56 * b, _pack(_dot(phi[b], _mat(*rows, jnp.zeros((8, DP), I32))) * LOG2E))

    others = [x_copy(c) for c in range(2, NC)] + w_copies
    store_values(0, 0, proj(wa[2], 0, xa[0]))
    wk_copy.wait()
    x_copy(1).wait()
    run([(cp.start,) for cp in others])
    load_x(1)
    for b in range(4):
        if b < 3:
            store_values(0, b + 1, proj(wa[2], b + 1, xa[0], (1, 3, 5)))
        fold(1, b)
    wq_copy.wait()
    background.append((pairs_a, pair_weights(wa, pairs_a, 2)))
    for b in range(4):
        store_features(phik[b], 0, proj(wa[1], b, xa[0]))
        fold(0, b)
    for b in range(4):
        store_features(phiq[0], b, proj(wa[0], b, xa[0], (1, 4)))
        a_kv(0, b)
    run([(cp.wait,) for cp in others])
    run([(load_x, 2)] + a_features(1))
    run([(load_x, 3)] + a_features(2))
    transpose(woa_in, woa, lambda x: x)
    transpose(wb_in, wb)
    background.append((pairs_b, pair_weights(wb, pairs_b, 0)))
    transpose(wob_in, wob, _attention_order)
    run(a_features(3))
    mix_and_attend(False)
    mix_and_attend(True)
    for c in range(NC):
        for b in range(4):
            out_copy(c, b).wait()


@jax.jit
def pallas_interleave_layers__linear_kernel_hedgehog__sliding_block__prompt_kernel(
    A_x: jax.Array,
    A_wqkv: jax.Array,
    A_w_phi: jax.Array,
    A_wo: jax.Array,
    B_x: jax.Array,
    B_wqkv: jax.Array,
    B_wo: jax.Array,
):
    del B_x
    vmem = pltpu.VMEM
    words = lambda rows: vmem((1, 4, rows + 8, 128), I32)
    out = pl.pallas_call(
        _kernel,
        out_shape=jax.ShapeDtypeStruct((D, S), A_x.dtype),
        in_specs=[pl.BlockSpec(memory_space=pl.ANY)] * 6,
        out_specs=pl.BlockSpec(memory_space=pl.ANY),
        scratch_shapes=[
            vmem((NC, D, T), BF16), vmem((D, 3 * D), BF16), vmem((D, DH), BF16), vmem((D, D), BF16),
            vmem((D, 3 * D), BF16), vmem((D, D), BF16), vmem((D, 128), F32), vmem((D, 128), F32),
            vmem((1, 8, 64, 128), F32), vmem((1, 8, 32, 128), I32), vmem((1, 4, 48, 128), I32), vmem((1, 4, 4, 8, 128), I32),
            pltpu.SemaphoreType.DMA((NC + 7,)), pltpu.SemaphoreType.DMA((4 * NC,)),
            [[words(D // 2)] * n for n in (3, 1, 3, 1)] + [[words(24 * 56)] * 2],
            [[words(rows)] * NC
             for rows in (D + 64, 512 + 16, 512 + 16, D, D // 2, D // 2, 2 * T, 256, D // 2)]
            + [[words(rows)] * (4 * NC) for rows in (112, 64)],
            [vmem((1, 4, 288, 128), I32)] * 32,
        ],
        compiler_params=pltpu.CompilerParams(vmem_limit_bytes=100 * 1024 * 1024, flags={"XLA_TPU_EVENLY_DISTRIBUTE_CRITICAL_NODES": True}),
    )(
        A_x[0].T, A_wqkv, jnp.transpose(A_w_phi, (1, 0, 2)).reshape(DH * H, DH), A_wo, B_wqkv, B_wo,
    )
    return out.T[None]
```
